```python
import os as _os
_os.environ.setdefault("JAX_PLATFORMS", "cpu")
import jax
import jax.numpy as jnp

def _softmax(x, axis=-1):
    return jax.nn.softmax(x, axis=axis)
def _gelu(x):
    return jax.nn.gelu(x, approximate=True)
def _silu(x):
    return jax.nn.silu(x)
def _sigmoid(x):
    return jax.nn.sigmoid(x)
def _layernorm(x, axis=-1, eps=1e-5):
    m = jnp.mean(x, axis=axis, keepdims=True)
    v = jnp.var(x, axis=axis, keepdims=True)
    return (x - m) / jnp.sqrt(v + eps)
def _scatter_add(tgt, idx, src, axis=0):
    return tgt.at[idx].add(src)
def _segment_sum(src, seg, n):
    return jax.ops.segment_sum(src, seg, n)
class _Rng:
    def __init__(self, key):
        self._k = key
    def _next(self):
        self._k, sub = jax.random.split(self._k)
        return sub
    def normal(self, shape):
        return jax.random.normal(self._next(), shape, dtype=jnp.bfloat16)
    def randint(self, lo, hi, shape):
        return jax.random.randint(self._next(), shape, lo, hi, dtype=jnp.int32)
    def uniform(self, shape, lo=0.0, hi=1.0):
        return jax.random.uniform(self._next(), shape, jnp.bfloat16, lo, hi)
    def permutation(self, n):
        return jax.random.permutation(self._next(), n)


kernel_name = 'concat_heads__gqa_block_cached__gqa_block_cached__near_ridge'

def setup_inputs():
    _rng = _Rng(jax.random.key(int.from_bytes(__import__("os").urandom(4), "little")))
    _w = (lambda a: (lambda t: t.astype(jnp.bfloat16) if jnp.issubdtype(t.dtype, jnp.floating) else t)(jnp.asarray(a)))
    def _A_setup():
        B, Sq, D = 8, 240, 640
        Hq, Hkv, Sk, Dh = 32, 32, 1024, 192
        assert Hq % Hkv == 0, (Hq, Hkv)
        return {
            "x": _w((lambda *s: _rng.normal(s) * 0.8)(B, Sq, D)),
            "k_cache": _w((lambda *s: _rng.normal(s) * 0.8)(B, Hkv, Sk, Dh)),
            "v_cache": _w((lambda *s: _rng.normal(s) * 0.05)(B, Hkv, Sk, Dh)),
            "wq": _w((lambda *s: _rng.normal(s) * 0.8)(D, Hq * Dh) * (D ** -0.5)),
            "wo": _w((lambda *s: _rng.normal(s) * 0.05)(Hq * Dh, D) * ((Hq * Dh) ** -0.5)),
        }
    _A_in = _A_setup()

    def _B_setup():
        B, Sq, D = 8, 240, 640
        Hq, Hkv, Sk, Dh = 32, 32, 1024, 192
        assert Hq % Hkv == 0, (Hq, Hkv)
        return {
            "x": _w((lambda *s: _rng.normal(s) * 0.8)(B, Sq, D)),
            "k_cache": _w((lambda *s: _rng.normal(s) * 0.8)(B, Hkv, Sk, Dh)),
            "v_cache": _w((lambda *s: _rng.normal(s) * 0.05)(B, Hkv, Sk, Dh)),
            "wq": _w((lambda *s: _rng.normal(s) * 0.8)(D, Hq * Dh) * (D ** -0.5)),
            "wo": _w((lambda *s: _rng.normal(s) * 0.05)(Hq * Dh, D) * ((Hq * Dh) ** -0.5)),
        }
    _B_in = _B_setup()

    return {
        "A_x": _A_in["x"],
        "A_k_cache": _A_in["k_cache"],
        "A_v_cache": _A_in["v_cache"],
        "A_wq": _A_in["wq"],
        "A_wo": _A_in["wo"],
        "B_x": _B_in["x"],
        "B_k_cache": _B_in["k_cache"],
        "B_v_cache": _B_in["v_cache"],
        "B_wq": _B_in["wq"],
        "B_wo": _B_in["wo"],
    }

def reference(A_x, A_k_cache, A_v_cache, A_wq, A_wo, B_x, B_k_cache, B_v_cache, B_wq, B_wo):
    def _A_ref(x, k_cache, v_cache, wq, wo):
        B, Sq, D = x.shape
        Hq, Dh = 32, 192
        Hkv = k_cache.shape[1]
        rep = Hq // Hkv
        q = (lambda x, *d: x.transpose(*d))((x @ wq).reshape(B, Sq, Hq, Dh), 0, 2, 1, 3)
        k = jnp.repeat(k_cache, rep, axis=1)
        v = jnp.repeat(v_cache, rep, axis=1)
        scores = jnp.einsum("bhqd,bhkd->bhqk", q, k) * (Dh ** -0.5)
        p = _softmax(scores, axis=-1)
        o = jnp.einsum("bhqk,bhkd->bhqd", p, v)
        return (lambda x, *d: x.transpose(*d))(o, 0, 2, 1, 3).reshape(B, Sq, Hq * Dh) @ wo

    def _B_ref(x, k_cache, v_cache, wq, wo):
        B, Sq, D = x.shape
        Hq, Dh = 32, 192
        Hkv = k_cache.shape[1]
        rep = Hq // Hkv
        q = (lambda x, *d: x.transpose(*d))((x @ wq).reshape(B, Sq, Hq, Dh), 0, 2, 1, 3)
        k = jnp.repeat(k_cache, rep, axis=1)
        v = jnp.repeat(v_cache, rep, axis=1)
        scores = jnp.einsum("bhqd,bhkd->bhqk", q, k) * (Dh ** -0.5)
        p = _softmax(scores, axis=-1)
        o = jnp.einsum("bhqk,bhkd->bhqd", p, v)
        return (lambda x, *d: x.transpose(*d))(o, 0, 2, 1, 3).reshape(B, Sq, Hq * Dh) @ wo

    a = _A_ref(A_x, A_k_cache, A_v_cache, A_wq, A_wo)
    b = _B_ref(B_x, B_k_cache, B_v_cache, B_wq, B_wo)
    return jnp.concatenate([a, b], axis=-1)
```

```python
import functools
import jax
import jax.numpy as jnp
import numpy as np
from jax import lax
import jax.experimental.pallas as pl
import jax.experimental.pallas.tpu as pltpu

B, SQ, D = 8, 240, 640
H, SK, DH = 32, 1024, 192
NP = H // 2
PW = 2 * DH
QSCALE = float(DH ** -0.5 * np.log2(np.e))
bf16 = jnp.bfloat16
f32 = jnp.float32


def _softmax_rows(s):
    m = jnp.max(s, axis=1, keepdims=True)
    e = jnp.exp2(s - m)
    l = jnp.sum(e, axis=1, keepdims=True)
    return (e * (1.0 / l)).astype(bf16)


def _pair(x, wq, kt, vt, wo):
    q = jnp.dot(x, wq, preferred_element_type=f32)
    q = (q * QSCALE).astype(bf16)
    lane = lax.broadcasted_iota(jnp.int32, (SQ, 128), 1)
    qm = q[:, 128:256]
    zero = jnp.zeros_like(qm)
    q0 = jnp.concatenate([q[:, 0:128], jnp.where(lane < 64, qm, zero)], axis=1)
    q1 = jnp.concatenate([jnp.where(lane >= 64, qm, zero), q[:, 256:384]], axis=1)
    s0 = jnp.dot(q0, kt[0:256], preferred_element_type=f32)
    s1 = jnp.dot(q1, kt[128:384], preferred_element_type=f32)
    p0 = _softmax_rows(s0)
    p1 = _softmax_rows(s1)
    nt = (((1,), (1,)), ((), ()))
    o0 = lax.dot_general(vt[0:192], p0, nt, preferred_element_type=f32)
    o1 = lax.dot_general(vt[192:384], p1, nt, preferred_element_type=f32)
    oT = jnp.concatenate([o0, o1], axis=0).astype(bf16)
    tn = (((0,), (0,)), ((), ()))
    return lax.dot_general(oT, wo, tn, preferred_element_type=f32)


def _kernel(xa, ka, va, wqa, woa, xb, kb, vb, wqb, wob, out, acc):
    hp = pl.program_id(0)
    b = pl.program_id(1)

    @pl.when(hp == 0)
    def _():
        acc[b] = jnp.zeros((SQ, 2 * D), f32)

    ra = _pair(xa[b], wqa[...], ka[...], va[...], woa[...])
    rb = _pair(xb[b], wqb[...], kb[...], vb[...], wob[...])
    acc[b, :, 0:D] += ra
    acc[b, :, D:2 * D] += rb

    @pl.when(hp == NP - 1)
    def _():
        out[...] = acc[b].astype(bf16)


@jax.jit
def pallas_concat_heads__gqa_block_cached__gqa_block_cached__near_ridge_kernel(
        A_x, A_k_cache, A_v_cache, A_wq, A_wo, B_x, B_k_cache, B_v_cache, B_wq, B_wo):
    def kvT(c):
        return jnp.swapaxes(c, 2, 3).reshape(B, NP, PW, SK)
    x_spec = pl.BlockSpec((B, SQ, D), lambda hp, b: (0, 0, 0))
    kv_spec = pl.BlockSpec((None, None, PW, SK), lambda hp, b: (b, hp, 0, 0))
    wq_spec = pl.BlockSpec((D, PW), lambda hp, b: (0, hp))
    wo_spec = pl.BlockSpec((PW, D), lambda hp, b: (hp, 0))
    return pl.pallas_call(
        _kernel,
        grid=(NP, B),
        in_specs=[x_spec, kv_spec, kv_spec, wq_spec, wo_spec] * 2,
        out_specs=pl.BlockSpec((None, SQ, 2 * D), lambda hp, b: (jnp.where(hp == NP - 1, b, 0), 0, 0)),
        out_shape=jax.ShapeDtypeStruct((B, SQ, 2 * D), bf16),
        scratch_shapes=[pltpu.VMEM((B, SQ, 2 * D), f32)],
        compiler_params=pltpu.CompilerParams(
            dimension_semantics=("arbitrary", "arbitrary"),
            vmem_limit_bytes=100 * 1024 * 1024,
        ),
    )(A_x, kvT(A_k_cache), kvT(A_v_cache), A_wq, A_wo,
      B_x, kvT(B_k_cache), kvT(B_v_cache), B_wq, B_wo)
```

```python
import jax
import jax.numpy as jnp
import numpy as np
from jax import lax
import jax.experimental.pallas as pl
import jax.experimental.pallas.tpu as pltpu

B, SQ, D = 8, 240, 640
H, SK, DH = 32, 1024, 192
NP = H // 2
PW = 2 * DH
NI = NP * B
U = 2
NBODY = NI // U
WB = ((B - 2) // U) * U
XS0 = 2 * U - 1
QSCALE = float(DH ** -0.5 * np.log2(np.e))
bf16 = jnp.bfloat16
f32 = jnp.float32
NT = (((1,), (1,)), ((), ()))
TN = (((0,), (0,)), ((), ()))

PROLOGUE = "+qa +ka0 +qb".split()
FIRST = [s.split() for s in (
    "-qa -ka0 -qb +va0 +kb0 QZ0 QZ1 +vb0 QK0 QK1 +x0 -va0 +wo SM0 PV0 WO0 -kb0 +ka1 QK2 +va1 SM1 PV1 WO1 "
    "QK3 -vb0 -x0 +kb1 +vb1 SM2 PV2 WO2 QP0 QP1 +x1 SM3 PV3 WO3",
    "-ka1 -va1 -wo +ka2 +va2 QK0 QK1 OP0 AC0 SM0 PV0 WO0 OP1 AC1 -kb1 -vb1 -x1 +kb2 +vb2 +x2 QK2 SM1 PV1 WO1 "
    "QK3 QP0 +all3 SM2 PV2 WO2 QP1 SM3 PV3 WO3",
    "-all2 QK0 QK1 OP0 AC0 +next SM0 PV0 WO0 OP1 AC1 QK2 SM1 PV1 WO1 QP0 QK3 SM2 PV2 WO2 QP1 SM3 PV3 WO3",
    "-all3 QK1 QK0 OP0 AC0 SM0 PV0 WO0 OP1 AC1 SM1 PV1 WO1 QP0 QK2 QK3 SM2 PV2 WO2 QP1 SM3 PV3 WO3",
)]
MID = [s.split() for s in (
    "QK0 DS0 QK1 SM0 PV0 QP0 OP0 AC0 WO0 OP1 AC1 SM1 PV1 WO1 QK2 QK3 SM2 PV2 WO2 QP1 SM3 PV3 WO3",
    "QK1 QK0 OP0 AC0 SM0 PV0 WO0 OP1 AC1 SM1 PV1 WO1 QP0 QK2 QK3 SM2 PV2 WO2 QP1 SM3 PV3 WO3",
)]
LAST = [s.split() for s in (
    "QK0 QK1 SM0 PV0 QP0 OP0 AC0 WO0 OP1 AC1 OT0 SM1 PV1 WO1 QK2 QK3 SM2 PV2 WO2 QP1 SM3 PV3 WO3",
    "QK1 QK0 OP0 AC0 SM0 PV0 WO0 OP1 AC1 OT0 SM1 PV1 WO1 QK2 QK3 OF0 SM2 PV2 WO2 SM3 PV3 WO3 OF1",
)]
NFIRST = len(FIRST) // U


def _qproj(x, wq, q_ref):
    q = jnp.dot(x, wq, preferred_element_type=f32)
    q = (q * QSCALE).astype(bf16)
    lane = lax.broadcasted_iota(jnp.int32, (SQ, 128), 1)
    qm = q[:, 128:256]
    zero = jnp.zeros_like(qm)
    q_ref[0, :, 0:128] = q[:, 0:128]
    q_ref[0, :, 128:256] = jnp.where(lane < 64, qm, zero)
    q_ref[1, :, 0:128] = jnp.where(lane >= 64, qm, zero)
    q_ref[1, :, 128:256] = q[:, 256:384]


def _exp(s):
    e = jnp.exp2(s - jnp.max(s, axis=1, keepdims=True))
    lp = e[:, 0:128]
    for j in range(1, SK // 128):
        lp = lp + e[:, j * 128:(j + 1) * 128]
    return e.astype(bf16), lp.astype(bf16)


def _pv(vt, p, lp):
    oT = lax.dot_general(vt, p, NT, preferred_element_type=f32)
    lT = lax.dot_general(jnp.ones((16, 128), bf16), lp, NT, preferred_element_type=f32)
    return (oT * (1.0 / lT[0:1])).astype(bf16)


def _oproj(oT_ref, wo):
    return lax.dot_general(oT_ref[...], wo, TN, preferred_element_type=f32)


def _kernel(xa_h, ka_h, va_h, wqa_h, woa_h, xb_h, kb_h, vb_h, wqb_h, wob_h, out_h,
            xbuf, kbuf, vbuf, wqs, wos, acc, qs, os_, stage,
            x_sem, kv_sem, w_sem, o_sem):
    x_h, k_h, v_h = (xa_h, xb_h), (ka_h, kb_h), (va_h, vb_h)
    wq_h, wo_h = (wqa_h, wqb_h), (woa_h, wob_h)

    def x_copy(r, n, slot):
        return pltpu.make_async_copy(x_h[r].at[n & (B - 1)], xbuf.at[r, slot], x_sem.at[r, slot])

    def k_copy(r, n, slot):
        return pltpu.make_async_copy(k_h[r].at[n & (B - 1), n >> 3], kbuf.at[r, slot], kv_sem.at[r, 0, slot])

    def v_copy(r, n, slot):
        return pltpu.make_async_copy(v_h[r].at[n & (B - 1), n >> 3], vbuf.at[r, slot], kv_sem.at[r, 1, slot])

    def xn_copy(r, n, slot):
        return x_copy(r, jnp.minimum(n + 1, NI - 1), slot)

    def wq_copy(r, g):
        src = wq_h[r].at[:, pl.ds(pl.multiple_of(g * PW, 128), PW)]
        return pltpu.make_async_copy(src, wqs.at[r, g], w_sem.at[r, 0, g & 1])

    def wo_copy(r, g):
        src = wo_h[r].at[pl.ds(pl.multiple_of(g * PW, 128), PW), :]
        return pltpu.make_async_copy(src, wos.at[r, g], w_sem.at[r, 1, g & 1])

    def w_copies(g):
        return [wq_copy(0, g), wq_copy(1, g), wo_copy(0, g), wo_copy(1, g)]

    def o_copy(b):
        return pltpu.make_async_copy(stage.at[b], out_h.at[b], o_sem.at[b])

    parts = {"ka": [(k_copy, 0)], "va": [(v_copy, 0)], "kb": [(k_copy, 1)], "vb": [(v_copy, 1)],
             "x": [(xn_copy, 0), (xn_copy, 1)]}
    parts["all"] = parts["ka"] + parts["va"] + parts["kb"] + parts["vb"] + parts["x"]

    def item_copies(n, slot, kind="all"):
        return [f(r, n, slot) for f, r in parts[kind]]

    def body_copies(S):
        return [c for i in range(U) for c in item_copies(S * U + i, (S & 1) * U + i)]

    def group(name):
        if name == "qa":
            return [x_copy(0, 0, XS0), wq_copy(0, 0)]
        if name == "qb":
            return [x_copy(1, 0, XS0), wq_copy(1, 0)]
        if name == "wo":
            return [wo_copy(0, 0), wo_copy(1, 0)]
        if name == "next":
            return body_copies(NFIRST)
        n = int(name[-1])
        return item_copies(n, n % (2 * U), name[:-1])

    def write_out(b):
        stage[b] = acc[b].astype(bf16)
        o_copy(b).start()

    def phases(s, slot, order, start_next=None):
        gn = jnp.minimum(s + 1, NI - 1) >> 3
        gp = jnp.maximum(s - 1, 0) >> 3
        bp = (s + B - 1) & (B - 1)
        live = {}
        for ph in order:
            if ph[0] in "+-":
                for c in group(ph[1:]):
                    c.start() if ph[0] == "+" else c.wait()
                continue
            kind, i = ph[:2], int(ph[2])
            r, j = (i // 2, i % 2) if kind in ("QK", "SM", "PV", "WO") else (i, None)
            if kind == "DS":
                start_next()
            elif kind == "QZ":
                _qproj(xbuf[r, XS0], wqs[r, 0], qs.at[r])
            elif kind == "QP":
                _qproj(xbuf[r, slot], wqs[r, gn], qs.at[r])
            elif kind == "QK":
                live["s", i] = jnp.dot(qs[r, j], kbuf[r, slot, 128 * j:128 * j + 256, :],
                                       preferred_element_type=f32)
            elif kind == "SM":
                live["p", i] = _exp(live.pop(("s", i)))
            elif kind == "PV":
                live["o", i] = _pv(vbuf[r, slot, DH * j:DH * j + DH, :], *live.pop(("p", i)))
            elif kind == "WO":
                os_[r, DH * j:DH * j + DH, :] = live.pop(("o", i))
            elif kind == "OP":
                live["r", r] = _oproj(os_.at[r], wos[r, gp])
            elif kind == "AC":
                acc[bp, :, r * D:(r + 1) * D] += live.pop(("r", r))
            elif kind == "OF":
                acc[B - 1, :, r * D:(r + 1) * D] += _oproj(os_.at[r], wos[r, NP - 1])
            elif kind == "OT":
                write_out(bp)
        assert not live

    def top_events(S):
        g, b0 = (S * U) >> 3, (S * U) & (B - 1)

        @pl.when(jnp.logical_or(g == 0, b0 == WB))
        def _():
            @pl.when(g == 0)
            def _():
                for i in range(U):
                    acc[b0 + i] = jnp.zeros((SQ, 2 * D), f32)

                @pl.when(b0 == 0)
                def _():
                    for c in w_copies(1):
                        c.start()

            @pl.when(b0 == WB)
            def _():
                @pl.when(g < NP - 1)
                def _():
                    for c in w_copies(g + 1):
                        c.wait()

                @pl.when(g < NP - 2)
                def _():
                    for c in w_copies(g + 2):
                        c.start()

    def bottom_events(S):
        @pl.when(S * U + U - 1 > NI - B)
        def _():
            for i in range(U):
                s = S * U + i

                @pl.when(s > NI - B)
                def _():
                    write_out((s + B - 1) & (B - 1))

    def mid_body(S, carry):
        top_events(S)
        for c in body_copies(S):
            c.wait()

        def start_next():
            for c in body_copies(S + 1):
                c.start()

        for i in range(U):
            phases(S * U + i, (S & 1) * U + i, MID[i], start_next)
        bottom_events(S)
        return carry

    for t in PROLOGUE:
        for c in group(t[1:]):
            c.start()
    for S in range(NFIRST):
        top_events(jnp.int32(S))
        for i in range(U):
            phases(S * U + i, (S & 1) * U + i, FIRST[S * U + i])

    lax.fori_loop(NFIRST, NBODY - 1, mid_body, 0)

    S = NBODY - 1
    for c in body_copies(S):
        c.wait()
    for i in range(U):
        phases(S * U + i, (S & 1) * U + i, LAST[i])
    write_out(B - 1)
    for b in range(B):
        o_copy(b).wait()


@jax.jit
def pallas_concat_heads__gqa_block_cached__gqa_block_cached__near_ridge_kernel(
        A_x, A_k_cache, A_v_cache, A_wq, A_wo, B_x, B_k_cache, B_v_cache, B_wq, B_wo):
    def kv_t(c):
        return jnp.swapaxes(c, 2, 3).reshape(B, NP, PW, SK)

    dma = pltpu.SemaphoreType.DMA
    return pl.pallas_call(
        _kernel,
        in_specs=[pl.BlockSpec(memory_space=pl.ANY)] * 10,
        out_specs=pl.BlockSpec(memory_space=pl.ANY),
        out_shape=jax.ShapeDtypeStruct((B, SQ, 2 * D), bf16),
        scratch_shapes=[
            pltpu.VMEM((2, 2 * U, SQ, D), bf16),
            pltpu.VMEM((2, 2 * U, PW, SK), bf16),
            pltpu.VMEM((2, 2 * U, PW, SK), bf16),
            pltpu.VMEM((2, NP, D, PW), bf16),
            pltpu.VMEM((2, NP, PW, D), bf16),
            pltpu.VMEM((B, SQ, 2 * D), f32),
            pltpu.VMEM((2, 2, SQ, 256), bf16),
            pltpu.VMEM((2, PW, SQ), bf16),
            pltpu.VMEM((B, SQ, 2 * D), bf16),
            dma((2, 2 * U)),
            dma((2, 2, 2 * U)),
            dma((2, 2, 2)),
            dma((B,)),
        ],
        compiler_params=pltpu.CompilerParams(vmem_limit_bytes=100 * 1024 * 1024),
    )(A_x, kv_t(A_k_cache), kv_t(A_v_cache), A_wq, A_wo,
      B_x, kv_t(B_k_cache), kv_t(B_v_cache), B_wq, B_wo)
```

```python
import jax
import jax.numpy as jnp
import numpy as np
from jax import lax
import jax.experimental.pallas as pl
import jax.experimental.pallas.tpu as pltpu

B, SQ, D = 8, 240, 640
H, SK, DH = 32, 1024, 192
NP = H // 2
PW = 2 * DH
NI = NP * B
U = 2
NBODY = NI // U
WB = ((B - 2) // U) * U
QSCALE = float(DH ** -0.5 * np.log2(np.e))
bf16 = jnp.bfloat16
f32 = jnp.float32
NT = (((1,), (1,)), ((), ()))
TN = (((0,), (0,)), ((), ()))

PROLOGUE = "+qa +ka0 +qb".split()
FIRST = [s.split() for s in (
    "-qa -ka0 -qb +va0 +kb0 QZ0 QZ1 ZA0 +vb0 QK0 QK1 +x1 -va0 +wo SM0 PV0 WO0 -kb0 +ka1 QK2 +va1 SM1 PV1 WO1 "
    "QK3 -vb0 -x1 +kb1 +vb1 SM2 PV2 WO2 QP0 QP1 +x2 SM3 PV3 WO3",
    "-ka1 -va1 -wo +ka2 +va2 ZA1 QK0 QK1 OP0 AC0 SM0 PV0 WO0 OP1 AC1 -kb1 -vb1 -x2 +kb2 +vb2 +x3 QK2 SM1 PV1 WO1 "
    "QK3 QP0 +kv3 +x4 SM2 PV2 WO2 QP1 SM3 PV3 WO3",
    "-kv2 -x3 ZA2 QK0 QK1 OP0 AC0 +next SM0 PV0 WO0 OP1 AC1 QK2 SM1 PV1 WO1 QP0 QK3 SM2 PV2 WO2 QP1 SM3 PV3 WO3",
    "-kv3 -x4 +x5 +x6 +x7 +w1 ZA3 QK1 QK0 OP0 AC0 SM0 PV0 WO0 OP1 AC1 SM1 PV1 WO1 QP0 QK2 QK3 SM2 PV2 WO2 QP1 SM3 PV3 WO3",
)]
MID = [s.split() for s in (
    "QK0 DS0 QK1 SM0 PV0 QP0 OP0 AC0 WO0 OP1 AC1 SM1 PV1 WO1 QK2 QK3 SM2 PV2 WO2 QP1 SM3 PV3 WO3",
    "QK1 QK0 OP0 AC0 SM0 PV0 WO0 OP1 AC1 SM1 PV1 WO1 QP0 QK2 QK3 SM2 PV2 WO2 QP1 SM3 PV3 WO3",
)]
LAST = [s.split() for s in (
    "QK0 QK1 SM0 PV0 QP0 OP0 AC0 WO0 OP1 AC1 OT0 SM1 PV1 WO1 QK2 QK3 SM2 PV2 WO2 QP1 SM3 PV3 WO3",
    "QK1 QK0 OP0 AC0 SM0 PV0 WO0 OP1 AC1 OT0 SM1 PV1 WO1 QK2 QK3 OF0 SM2 PV2 WO2 SM3 PV3 WO3 OF1",
)]
NFIRST = len(FIRST) // U


def _qproj(x, wq, q_ref):
    q = jnp.dot(x, wq, preferred_element_type=f32)
    q = (q * QSCALE).astype(bf16)
    lane = lax.broadcasted_iota(jnp.int32, (SQ, 128), 1)
    qm = q[:, 128:256]
    zero = jnp.zeros_like(qm)
    q_ref[0, :, 0:128] = q[:, 0:128]
    q_ref[0, :, 128:256] = jnp.where(lane < 64, qm, zero)
    q_ref[1, :, 0:128] = jnp.where(lane >= 64, qm, zero)
    q_ref[1, :, 128:256] = q[:, 256:384]


def _exp(s):
    e = jnp.exp2(s - jnp.max(s, axis=1, keepdims=True))
    p = e.astype(bf16)
    lp = e[:, 0:128]
    for j in range(1, SK // 128):
        lp = lp + e[:, j * 128:(j + 1) * 128]
    return p, lp.astype(bf16)


def _pv(vt, p, lp):
    ones = jnp.ones((16, 128), bf16)
    oT = lax.dot_general(vt, p, NT, preferred_element_type=f32)
    lT = lax.dot_general(ones, lp, NT, preferred_element_type=f32)
    return (oT * (1.0 / lT[0:1])).astype(bf16)


def _oproj(oT_ref, wo):
    return lax.dot_general(oT_ref[...], wo, TN, preferred_element_type=f32)


def _kernel(xa_h, ka_h, va_h, wqa_h, woa_h, xb_h, kb_h, vb_h, wqb_h, wob_h, out_h,
            xbuf, kvbuf, wqs, wos, acc, qs, os_, stage,
            x_sem, kv_sem, ring_sem, w_sem, o_sem):
    x_h, k_h, v_h = (xa_h, xb_h), (ka_h, kb_h), (va_h, vb_h)
    wq_h, wo_h = (wqa_h, wqb_h), (woa_h, wob_h)

    def x_copy(r, b):
        return pltpu.make_async_copy(x_h[r].at[b], xbuf.at[r, b], x_sem.at[r, b])

    def kv_copy(src, kind, r, n, par, i, sem):
        return pltpu.make_async_copy(src[r].at[n & (B - 1), n >> 3], kvbuf.at[par, i, r, kind], sem)

    def wq_copy(r, g):
        src = wq_h[r].at[:, pl.ds(pl.multiple_of(g * PW, 128), PW)]
        return pltpu.make_async_copy(src, wqs.at[r, g], w_sem.at[r, 0, g & 1])

    def wo_copy(r, g):
        src = wo_h[r].at[pl.ds(pl.multiple_of(g * PW, 128), PW), :]
        return pltpu.make_async_copy(src, wos.at[r, g], w_sem.at[r, 1, g & 1])

    def w_copies(g):
        return [wq_copy(0, g), wq_copy(1, g), wo_copy(0, g), wo_copy(1, g)]

    def o_copy(b):
        return pltpu.make_async_copy(stage.at[b], out_h.at[b], o_sem.at[b])

    parts = {"ka": [(k_h, 0, 0)], "va": [(v_h, 1, 0)], "kb": [(k_h, 0, 1)], "vb": [(v_h, 1, 1)]}
    parts["kv"] = parts["ka"] + parts["va"] + parts["kb"] + parts["vb"]

    def item_copies(n, kind):
        par, i = (n // U) & 1, n % U
        return [kv_copy(src, kd, r, n, par, i, kv_sem.at[n, r, kd]) for src, kd, r in parts[kind]]

    def ring_start(S, par):
        for i in range(U):
            n = jnp.minimum(S * U + i, NI - 1)
            for src, kd, r in parts["kv"]:
                kv_copy(src, kd, r, n, par, i, ring_sem.at[par]).start()

    def ring_wait(par):
        pltpu.make_async_copy(kvbuf.at[par], kvbuf.at[par], ring_sem.at[par]).wait()

    def group(name):
        kind = name.rstrip("0123456789")
        n = int(name[len(kind):] or 0)
        if kind == "qa":
            return [x_copy(0, 0), wq_copy(0, 0)]
        if kind == "qb":
            return [x_copy(1, 0), wq_copy(1, 0)]
        if kind == "wo":
            return [wo_copy(0, 0), wo_copy(1, 0)]
        if kind == "w":
            return w_copies(n)
        if kind == "x":
            return [x_copy(0, n), x_copy(1, n)]
        return item_copies(n, kind)

    def write_out(b):
        stage[b] = acc[b].astype(bf16)
        o_copy(b).start()

    def phases(s, par, si, order, start_next=None):
        gn = jnp.minimum(s + 1, NI - 1) >> 3
        gp = jnp.maximum(s - 1, 0) >> 3
        bp = (s + B - 1) & (B - 1)
        live = {}
        for ph in order:
            if ph == "+next":
                ring_start(NFIRST, NFIRST & 1)
                continue
            if ph[0] in "+-":
                for c in group(ph[1:]):
                    c.start() if ph[0] == "+" else c.wait()
                continue
            kind, i = ph[:2], int(ph[2])
            r, j = (i // 2, i % 2) if kind in ("QK", "SM", "PV", "WO") else (i, None)
            if kind == "DS":
                start_next()
            elif kind == "ZA":
                acc[i] = jnp.zeros((SQ, 2 * D), f32)
            elif kind == "QZ":
                _qproj(xbuf[r, 0], wqs[r, 0], qs.at[r])
            elif kind == "QP":
                _qproj(xbuf[r, (s + 1) & (B - 1)], wqs[r, gn], qs.at[r])
            elif kind == "QK":
                live["s", i] = jnp.dot(qs[r, j], kvbuf[par, si, r, 0, 128 * j:128 * j + 256, :],
                                       preferred_element_type=f32)
            elif kind == "SM":
                live["p", i] = _exp(live.pop(("s", i)))
            elif kind == "PV":
                live["o", i] = _pv(kvbuf[par, si, r, 1, DH * j:DH * j + DH, :], *live.pop(("p", i)))
            elif kind == "WO":
                os_[r, DH * j:DH * j + DH, :] = live.pop(("o", i))
            elif kind == "OP":
                live["r", r] = _oproj(os_.at[r], wos[r, gp])
            elif kind == "AC":
                acc[bp, :, r * D:(r + 1) * D] += live.pop(("r", r))
            elif kind == "OF":
                acc[B - 1, :, r * D:(r + 1) * D] += _oproj(os_.at[r], wos[r, NP - 1])
            elif kind == "OT":
                write_out(bp)
        assert not live

    def top_events(S):
        g, b0 = (S * U) >> 3, (S * U) & (B - 1)
        late = S * U > NI - B

        @pl.when(jnp.logical_or(jnp.logical_or(g == 0, b0 == WB), late))
        def _():
            @pl.when(g == 0)
            def _():
                for i in range(U):
                    acc[b0 + i] = jnp.zeros((SQ, 2 * D), f32)
                for r in range(2):
                    x_copy(r, b0 + 1).wait()

                @pl.when(b0 + U < B)
                def _():
                    for r in range(2):
                        x_copy(r, jnp.minimum(b0 + U, B - 1)).wait()

            @pl.when(b0 == WB)
            def _():
                @pl.when(g < NP - 1)
                def _():
                    for c in w_copies(g + 1):
                        c.wait()

                @pl.when(g < NP - 2)
                def _():
                    for c in w_copies(g + 2):
                        c.start()

            @pl.when(late)
            def _():
                @pl.when(b0 > U)
                def _():
                    write_out(b0 - U - 1)

                write_out(b0 - U)

    def mid_body(S, carry):
        top_events(S)
        par = S & 1
        ring_wait(par)

        def start_next():
            ring_start(S + 1, 1 - par)

        for i in range(U):
            phases(S * U + i, par, i, MID[i], start_next)
        return carry

    for t in PROLOGUE:
        for c in group(t[1:]):
            c.start()
    for n, order in enumerate(FIRST):
        phases(n, (n // U) & 1, n % U, order)

    lax.fori_loop(NFIRST, NBODY - 1, mid_body, 0)

    S = NBODY - 1
    ring_wait(S & 1)
    write_out(B - 2 * U - 1)
    write_out(B - 2 * U)
    for i in range(U):
        phases(S * U + i, S & 1, i, LAST[i])
    write_out(B - 1)
    for b in range(B):
        o_copy(b).wait()


@jax.jit
def pallas_concat_heads__gqa_block_cached__gqa_block_cached__near_ridge_kernel(
        A_x, A_k_cache, A_v_cache, A_wq, A_wo, B_x, B_k_cache, B_v_cache, B_wq, B_wo):
    def kv_t(c):
        return jnp.swapaxes(c, 2, 3).reshape(B, NP, PW, SK)

    dma = pltpu.SemaphoreType.DMA
    return pl.pallas_call(
        _kernel,
        in_specs=[pl.BlockSpec(memory_space=pl.ANY)] * 10,
        out_specs=pl.BlockSpec(memory_space=pl.ANY),
        out_shape=jax.ShapeDtypeStruct((B, SQ, 2 * D), bf16),
        scratch_shapes=[
            pltpu.VMEM((2, B, SQ, D), bf16),
            pltpu.VMEM((2, U, 2, 2, PW, SK), bf16),
            pltpu.VMEM((2, NP, D, PW), bf16),
            pltpu.VMEM((2, NP, PW, D), bf16),
            pltpu.VMEM((B, SQ, 2 * D), f32),
            pltpu.VMEM((2, 2, SQ, 256), bf16),
            pltpu.VMEM((2, PW, SQ), bf16),
            pltpu.VMEM((B, SQ, 2 * D), bf16),
            dma((2, B)),
            dma((len(FIRST), 2, 2)),
            dma((2,)),
            dma((2, 2, 2)),
            dma((B,)),
        ],
        compiler_params=pltpu.CompilerParams(vmem_limit_bytes=100 * 1024 * 1024),
    )(A_x, kv_t(A_k_cache), kv_t(A_v_cache), A_wq, A_wo,
      B_x, kv_t(B_k_cache), kv_t(B_v_cache), B_wq, B_wo)
```
